```python
import os as _os
_os.environ.setdefault("JAX_PLATFORMS", "cpu")
import jax
import jax.numpy as jnp

def _softmax(x, axis=-1):
    return jax.nn.softmax(x, axis=axis)
def _gelu(x):
    return jax.nn.gelu(x, approximate=True)
def _silu(x):
    return jax.nn.silu(x)
def _sigmoid(x):
    return jax.nn.sigmoid(x)
def _layernorm(x, axis=-1, eps=1e-5):
    m = jnp.mean(x, axis=axis, keepdims=True)
    v = jnp.var(x, axis=axis, keepdims=True)
    return (x - m) / jnp.sqrt(v + eps)
def _scatter_add(tgt, idx, src, axis=0):
    return tgt.at[idx].add(src)
def _segment_sum(src, seg, n):
    return jax.ops.segment_sum(src, seg, n)
class _Rng:
    def __init__(self, key):
        self._k = key
    def _next(self):
        self._k, sub = jax.random.split(self._k)
        return sub
    def normal(self, shape):
        return jax.random.normal(self._next(), shape, dtype=jnp.bfloat16)
    def randint(self, lo, hi, shape):
        return jax.random.randint(self._next(), shape, lo, hi, dtype=jnp.int32)
    def uniform(self, shape, lo=0.0, hi=1.0):
        return jax.random.uniform(self._next(), shape, jnp.bfloat16, lo, hi)
    def permutation(self, n):
        return jax.random.permutation(self._next(), n)


kernel_name = 'interleave_layers__sliding_block__mha_block__prompt'

def setup_inputs():
    _rng = _Rng(jax.random.key(int.from_bytes(__import__("os").urandom(4), "little")))
    _w = (lambda a: (lambda t: t.astype(jnp.bfloat16) if jnp.issubdtype(t.dtype, jnp.floating) else t)(jnp.asarray(a)))
    def _A_setup():
        B, S, D = 1, 2048, 512
        return {
            "x": _w((lambda *s: _rng.normal(s) * 0.05)(B, S, D)),
            "wqkv": _w((lambda *s: _rng.normal(s) * 0.05)(D, 3 * D)),
            "wo": _w((lambda *s: _rng.normal(s) * 0.05)(D, D)),
        }
    _A_in = _A_setup()

    def _B_setup():
        B, S, D, H = 1, 2048, 512, 32
        return {
            "x": _w((lambda *s: _rng.normal(s) * 0.05)(B, S, D)),
            "wqkv": _w((lambda *s: _rng.normal(s) * 0.05)(D, 3 * D)),
            "wo": _w((lambda *s: _rng.normal(s) * 0.05)(D, D)),
        }
    _B_in = _B_setup()

    return {
        "A_x": _A_in["x"],
        "A_wqkv": _A_in["wqkv"],
        "A_wo": _A_in["wo"],
        "B_x": _B_in["x"],
        "B_wqkv": _B_in["wqkv"],
        "B_wo": _B_in["wo"],
    }

def reference(A_x, A_wqkv, A_wo, B_x, B_wqkv, B_wo):
    def _A_ref(x, wqkv, wo):
        B, S, D = x.shape
        H = 32; Dh = D // H; W = 256
        qkv = (lambda x, *d: x.transpose(*d))((x @ wqkv).reshape(B, S, 3, H, Dh), 2, 0, 3, 1, 4)
        q, k, v = qkv[0], qkv[1], qkv[2]
        scores = jnp.einsum("bhqd,bhkd->bhqk", q, k) * (Dh ** -0.5)
        idx = jnp.arange(S)
        mask = (idx[:, None] - idx[None, :] >= 0) & (idx[:, None] - idx[None, :] < W)
        scores = jnp.where(mask[None, None], scores, -1e9)
        p = _softmax(scores, axis=-1)
        o = jnp.einsum("bhqk,bhkd->bhqd", p, v)
        return (lambda x, *d: x.transpose(*d))(o, 0, 2, 1, 3).reshape(B, S, D) @ wo

    def _B_ref(x, wqkv, wo):
        B, S, D = x.shape
        H = 32
        Dh = D // H
        qkv = (lambda x, *d: x.transpose(*d))((x @ wqkv).reshape(B, S, 3, H, Dh), 2, 0, 3, 1, 4)
        q, k, v = qkv[0], qkv[1], qkv[2]
        scores = jnp.einsum("bhqd,bhkd->bhqk", q, k) * (Dh ** -0.5)
        p = _softmax(scores, axis=-1)
        o = jnp.einsum("bhqk,bhkd->bhqd", p, v)
        return (lambda x, *d: x.transpose(*d))(o, 0, 2, 1, 3).reshape(B, S, D) @ wo

    x = A_x
    x = x + _A_ref(_layernorm(x, axis=-1), A_wqkv, A_wo)
    x = x + _B_ref(_layernorm(x, axis=-1), B_wqkv, B_wo)
    x = x + _A_ref(_layernorm(x, axis=-1), A_wqkv, A_wo)
    x = x + _B_ref(_layernorm(x, axis=-1), B_wqkv, B_wo)
    return x
```

```python
import functools
import math

import jax
import jax.numpy as jnp
import jax.experimental.pallas as pl
import jax.experimental.pallas.tpu as pltpu

S, D, H, DH, WIN = 2048, 512, 32, 16, 256
F32, BF16 = jnp.float32, jnp.bfloat16
QSCALE = (DH ** -0.5) * math.log2(math.e)
NEG = -1e30
RC = 256
NRC = S // RC
TQ = 512
NSUB = 4
NT = (((1,), (1,)), ((), ()))


def _kernel(x_in, wk_in, wqv_in, wo_in, out_ref,
            x_s, xn_s, k_s, qp_s, vt_s, ot_s, sf_s, mf_s, sw_s, mw_s, bias_s):
    qp_s[...] = jnp.zeros_like(qp_s)
    kk = jax.lax.broadcasted_iota(jnp.int32, (128, 128), 0)
    qq = jax.lax.broadcasted_iota(jnp.int32, (128, 128), 1)
    zero = jnp.zeros((128, 128), F32)
    neg = jnp.full((128, 128), NEG, F32)
    upper = jnp.where(kk > qq, zero, neg)
    lower = jnp.where(kk <= qq, zero, neg)
    for v in range(3):
        bias_s[v, 0] = upper if v >= 2 else neg
        bias_s[v, 1] = zero if v >= 1 else neg
        bias_s[v, 2] = lower

    def rows(c):
        return pl.ds(pl.multiple_of(c * RC, RC), RC)

    def layernorm(x):
        mu = jnp.mean(x, axis=-1, keepdims=True)
        xc = x - mu
        var = jnp.mean(xc * xc, axis=-1, keepdims=True)
        return (xc * jax.lax.rsqrt(var + 1e-5)).astype(BF16)

    def project(c, w):
        xn = xn_s[rows(c), :]
        k = jnp.dot(xn, wk_in[w], preferred_element_type=F32).astype(BF16)
        for g in range(4):
            k_s[g, rows(c), :] = k[:, g * 128:(g + 1) * 128]
        qv = jax.lax.dot_general(wqv_in[w], xn, NT, preferred_element_type=F32)
        q = (qv[:D] * QSCALE).astype(BF16)
        for h in range(H):
            r = (h % 8) * 16
            qp_s[h, r:r + 16, rows(c)] = q[h * 16:(h + 1) * 16]
        vt_s[:, rows(c)] = qv[D:].astype(BF16)

    def outproj(c, w):
        o = ot_s[:, rows(c)].T.astype(BF16)
        return x_s[rows(c), :] + jnp.dot(o, wo_in[w], preferred_element_type=F32)

    def colmax(m, s):
        for i in range(s.shape[0] // 8):
            x = s[i * 8:(i + 1) * 8]
            m = x if m is None else jnp.maximum(m, x)
        return m

    def colsum_rev(l, p):
        for i in reversed(range(p.shape[0] // 8)):
            x = p[i * 8:(i + 1) * 8]
            l = x if l is None else l + x
        return l

    def bmax(m):
        return jnp.broadcast_to(jnp.max(m, axis=0, keepdims=True), m.shape)

    def full_attention():
        nq = S // TQ
        nu = H * nq
        nc = S // 128

        def a_chunk(u, j, c, m):
            h = u // nq
            qb = u % nq
            w = qp_s[h, :, pl.ds(pl.multiple_of(qb * TQ, TQ), TQ)]
            s = jnp.dot(k_s[h // 8, c * 128:(c + 1) * 128, :], w, preferred_element_type=F32)
            sf_s[j, c * 128:(c + 1) * 128, :] = s
            return colmax(m, s)

        for j in range(NSUB):
            m = None
            for c in range(nc):
                m = a_chunk(j, j, c, m)
            mf_s[j] = bmax(m)

        def body(i, carry):
            for j in range(NSUB):
                ub = NSUB * i + j
                ua = jnp.minimum(ub + NSUB, nu - 1)
                h = ub // nq
                qb = ub % nq
                hrow = pl.ds(pl.multiple_of(h * 16, 16), 16)
                mb = mf_s[j][0:1, :]
                ma = l = o = None
                for c in range(nc):
                    p = jnp.exp2(sf_s[j, c * 128:(c + 1) * 128, :] - mb)
                    l = colsum_rev(l, p)
                    p = p.astype(BF16)
                    ma = a_chunk(ua, j, c, ma)
                    co = jnp.dot(vt_s[hrow, c * 128:(c + 1) * 128], p, preferred_element_type=F32)
                    o = co if o is None else co + o
                mf_s[j] = bmax(ma)
                lsum = jnp.sum(l, axis=0, keepdims=True)
                ot_s[hrow, pl.ds(pl.multiple_of(qb * TQ, TQ), TQ)] = o / lsum
            return carry
        jax.lax.fori_loop(0, nu // NSUB, body, 0)

    def window_attention():
        nb = S // 128

        def blk(b):
            return pl.ds(pl.multiple_of(b * 128, 128), 128)

        def a_chunk(i, quad, c, m):
            w = jnp.concatenate([qp_s[quad * 4 + t, :, blk(i)] for t in range(4)], axis=1)
            kb = jnp.maximum(i - 2 + c, 0)
            s = jnp.dot(k_s[quad // 2, blk(kb), :], w, preferred_element_type=F32)
            b = bias_s[jnp.minimum(i, 2), c]
            s = s + jnp.concatenate([b] * 4, axis=1)
            sw_s[quad, c * 128:(c + 1) * 128, :] = s
            return colmax(m, s)

        for quad in range(8):
            m = None
            for c in range(3):
                m = a_chunk(0, quad, c, m)
            mw_s[quad] = bmax(m)

        def body(i, carry):
            ia = jnp.minimum(i + 1, nb - 1)
            for quad in range(8):
                mb = mw_s[quad][0:1, :]
                ma = l = None
                o = [None] * 4
                for c in range(3):
                    p = jnp.exp2(sw_s[quad, c * 128:(c + 1) * 128, :] - mb)
                    l = colsum_rev(l, p)
                    p = p.astype(BF16)
                    ma = a_chunk(ia, quad, c, ma)
                    kb = jnp.maximum(i - 2 + c, 0)
                    for t in range(4):
                        h = quad * 4 + t
                        co = jnp.dot(vt_s[h * 16:(h + 1) * 16, blk(kb)], p[:, t * 128:(t + 1) * 128],
                                     preferred_element_type=F32)
                        o[t] = co if o[t] is None else co + o[t]
                mw_s[quad] = bmax(ma)
                lsum = jnp.sum(l, axis=0, keepdims=True)
                for t in range(4):
                    h = quad * 4 + t
                    ot_s[h * 16:(h + 1) * 16, blk(i)] = o[t] / lsum[:, t * 128:(t + 1) * 128]
            return carry
        jax.lax.fori_loop(0, nb, body, 0)

    def first(c, carry):
        x = x_in[rows(c), :].astype(F32)
        x_s[rows(c), :] = x
        xn_s[rows(c), :] = layernorm(x)
        project(c, 0)
        return carry
    jax.lax.fori_loop(0, NRC, first, 0)

    def layer(l, carry):
        w = l % 2

        @pl.when(w == 0)
        def _():
            window_attention()

        @pl.when(w == 1)
        def _():
            full_attention()

        @pl.when(l < 3)
        def _():
            def mid(c, carry):
                x = outproj(c, w)
                x_s[rows(c), :] = x
                xn_s[rows(c), :] = layernorm(x)
                project(c, 1 - w)
                return carry
            jax.lax.fori_loop(0, NRC, mid, 0)
        return carry
    jax.lax.fori_loop(0, 4, layer, 0)

    def last(c, carry):
        out_ref[rows(c), :] = outproj(c, 1).astype(BF16)
        return carry
    jax.lax.fori_loop(0, NRC, last, 0)


@jax.jit
def pallas_interleave_layers__sliding_block__mha_block__prompt_kernel(A_x, A_wqkv, A_wo, B_x, B_wqkv, B_wo):
    del B_x
    x = A_x.reshape(S, D)
    wk = jnp.stack([A_wqkv[:, D:2 * D], B_wqkv[:, D:2 * D]])
    wqv = jnp.stack([jnp.concatenate([w[:, :D], w[:, 2 * D:]], axis=1).T for w in (A_wqkv, B_wqkv)])
    wo = jnp.stack([A_wo, B_wo])
    out = pl.pallas_call(
        _kernel,
        out_shape=jax.ShapeDtypeStruct((S, D), BF16),
        scratch_shapes=[
            pltpu.VMEM((S, D), F32),
            pltpu.VMEM((S, D), BF16),
            pltpu.VMEM((4, S, 128), BF16),
            pltpu.VMEM((H, 128, S), BF16),
            pltpu.VMEM((D, S), BF16),
            pltpu.VMEM((D, S), F32),
            pltpu.VMEM((NSUB, S, TQ), F32),
            pltpu.VMEM((NSUB, 8, TQ), F32),
            pltpu.VMEM((8, 384, 512), F32),
            pltpu.VMEM((8, 8, 512), F32),
            pltpu.VMEM((3, 3, 128, 128), F32),
        ],
        compiler_params=pltpu.CompilerParams(vmem_limit_bytes=110 * 1024 * 1024),
        name="fused4",
    )(x, wk, wqv, wo)
    return out.reshape(1, S, D)
```

```python
import math

import jax
import jax.numpy as jnp
import jax.experimental.pallas as pl
import jax.experimental.pallas.tpu as pltpu

S, D, H, DH, WIN = 2048, 512, 32, 16, 256
F32, BF16, I32, I8, U32 = jnp.float32, jnp.bfloat16, jnp.int32, jnp.int8, jnp.uint32
QSCALE = (DH ** -0.5) * math.log2(math.e)
NEG = -1e30
RC = 256
NRC = S // RC
CPI = 2
NX = NRC // CPI
TQ = 512
KC = 256
NSUB = 16
NHW = 8
WLAG = 1
RG = 2
NB = S // 128
NT = (((1,), (1,)), ((), ()))
FRAC = 64.0
TMAX = 127.0 * FRAC
MAGIC = 12582912.0
TINY = 1e-30
RK = 6.0
L_LO, L_HI, O_HI = 2.0 ** -40, 2.0 ** 40, 3e38


def _recip(x):
    r = pl.reciprocal(x, approx=True)
    return r * (2.0 - x * r)


def _limbs(t):
    u32 = pltpu.bitcast(t + (MAGIC + 32.0), I32)
    h = u32 >> 6
    bl = u32 & 63
    b = bl - 32
    d = (bl - 28) >> 3
    u512 = u32 + 480
    a = u512 >> 10
    c = ((u512 & 1023) - 448) >> 7
    return h, a, b, c, d


def _kernel(x_hbm, wa_hbm, woa_hbm, wb_hbm, wob_hbm, out_hbm,
            xio_s, wraw_s, woraw_s, wk_s, wqv_s, wo_s, kinv_s, acol_s,
            kt_s, k8_s, q8_s, sc_s, vt_s, ot_s, msk_s, stat_s, sf_s, sems, *halves):
    x_s = halves[0:CPI]
    xn_s = halves[CPI:2 * CPI]
    XR = RC * CPI

    def xrows(i):
        return pl.ds(pl.multiple_of(i * XR, XR), XR)

    def x_copy(i):
        return pltpu.make_async_copy(x_hbm.at[xrows(i), :], xio_s.at[xrows(i), :], sems.at[4 + i])

    def out_copy(i):
        return pltpu.make_async_copy(xio_s.at[xrows(i), :], out_hbm.at[xrows(i), :], sems.at[4 + i])

    w_copies = [pltpu.make_async_copy(wa_hbm, wraw_s.at[0], sems.at[0]),
                pltpu.make_async_copy(wb_hbm, wraw_s.at[1], sems.at[1]),
                pltpu.make_async_copy(woa_hbm, woraw_s.at[0], sems.at[2]),
                pltpu.make_async_copy(wob_hbm, woraw_s.at[1], sems.at[3])]
    w_copies[0].start()
    for i in range(NX):
        x_copy(i).start()
    for cp in w_copies[1:]:
        cp.start()

    def packed(v):
        return pltpu.bitcast(v, U32)

    def unpacked(v):
        return pltpu.bitcast(v, BF16)

    kk = jax.lax.broadcasted_iota(I32, (128, 128), 0)
    qq = jax.lax.broadcasted_iota(I32, (128, 128), 1)
    msk_s[0] = jnp.where(kk <= qq, -1, 0)
    ks = jax.lax.broadcasted_iota(I32, (128, 128), 0) * 2
    msk_s[1] = jnp.where(ks <= qq, 0xFFFF, 0) | jnp.where(ks + 1 <= qq, -65536, 0)

    def prep_qkv(w):
        wk = wraw_s[w, :, D:2 * D]
        wk_s[w] = packed(wk)
        wkf = wk.astype(F32)
        alpha = jnp.maximum(jnp.sqrt(jnp.sum(wkf * wkf, axis=0, keepdims=True)), TINY)
        kinv_s[w] = jnp.broadcast_to((TMAX / RK) / alpha, (8, D))
        acol_s[w] = jnp.broadcast_to(alpha * (QSCALE / TMAX), (128, D)).T
        wqv_s[w, 0:D // 2] = packed(wraw_s[w, :, 0:D].astype(F32).T.astype(BF16))
        wqv_s[w, D // 2:D] = packed(wraw_s[w, :, 2 * D:3 * D].astype(F32).T.astype(BF16))

    def rows(c):
        return pl.ds(pl.multiple_of(c * RC, RC), RC)

    def layernorm(x):
        mu = jnp.mean(x, axis=-1, keepdims=True)
        xc = x - mu
        var = jnp.mean(xc * xc, axis=-1, keepdims=True)
        return (xc * jax.lax.rsqrt(var + 1e-5)).astype(BF16)

    def colacc(op, m, s):
        for i in range(s.shape[0] // 8):
            x = s[i * 8:(i + 1) * 8]
            m = x if m is None else op(m, x)
        return m

    def cols(c, n):
        return pl.ds(pl.multiple_of(c * RC + n * 128, 128), 128)

    def xtile(i, t, n):
        return unpacked(xn_s[t][i, n * 64:(n + 1) * 64, :])

    def k_limbs(t32, g, r32):
        lane_blk = jax.lax.broadcasted_iota(I32, (8, 128), 1) >> 4
        hk, ak, bk, ck, dk = [pltpu.bitcast(z.astype(I8), I32) for z in _limbs(t32)]
        kslots = (hk, hk, hk, hk, bk, ak, dk, ck)
        xs = [v if j == 0 else pltpu.roll(v, 16 * j, 1) for j, v in enumerate(kslots)]
        for s in range(3):
            bit = (lane_blk & (1 << s)) != 0
            xs = [jnp.where(bit, xs[(j + (1 << s)) % 8], xs[j]) for j in range(8)]
        for e in range(8):
            k8_s[g * 8 + e, r32, :] = pltpu.bitcast(xs[(-e) % 8], I8)

    def proj_k(i, t, w):
        c = i * CPI + t
        for g in range(4):
            gl = slice(g * 128, (g + 1) * 128)
            k = jnp.dot(unpacked(xn_s[t][i]), unpacked(wk_s[w, :, gl]), preferred_element_type=F32)
            kt = k * kinv_s[w, 0:1, gl]
            kt_s[rows(c), gl] = kt
            stat_s[0] = colacc(jnp.maximum, stat_s[0], jnp.abs(kt))
            for sl in range(RC // 32):
                k_limbs(kt[sl * 32:(sl + 1) * 32], g, pl.ds(pl.multiple_of(c * RC + sl * 32, 32), 32))

    def proj_v(i, t, w):
        for n in range(RC // 128):
            v = jax.lax.dot_general(unpacked(wqv_s[w, D // 2:D]), xtile(i, t, n), NT, preferred_element_type=F32)
            vt_s[:, cols(i * CPI + t, n)] = packed(v.astype(BF16))

    def proj_q(i, t, w):
        c = i * CPI + t
        for n in range(RC // 128):
            q = jax.lax.dot_general(unpacked(wqv_s[w, 0:D // 2]), xtile(i, t, n), NT, preferred_element_type=F32)
            q = (q * acol_s[w]).reshape(H, DH, 128)
            qm = jnp.maximum(jnp.max(jnp.abs(q), axis=1, keepdims=True), TINY)
            qi = pl.reciprocal(qm, approx=True)
            qm = qm * (2.0 - qm * qi)
            sc_s[:, :, cols(c, n)] = jnp.broadcast_to(qm * (RK * FRAC / (4.0 * 127.0)), (H, 8, 128))
            hq, aq, bq, cq, dq = _limbs(q * (qi * TMAX))
            qslots = (hq, hq, hq, hq, aq, bq, cq, dq)
            for h in range(H):
                blocks = [qslots[(beta - h) % 8][h] for beta in range(8)]
                q8_s[h, :, cols(c, n)] = jnp.concatenate(blocks, axis=0).astype(I8)

    def project(i, w):
        for t in range(CPI):
            proj_v(i, t, w)
            proj_k(i, t, w)
            proj_q(i, t, w)

    def check_k_range():
        tm = jnp.max(jnp.max(stat_s[0], axis=1, keepdims=True), axis=0, keepdims=True)
        stat_s[0] = jnp.zeros((8, 128), F32)
        stat_s[1] = jnp.full((8, 128), 1.0, F32)
        stat_s[2] = jnp.full((8, 128), 1.0, F32)
        stat_s[3] = jnp.zeros((8, 128), F32)
        tms = tm[0, 0]

        @pl.when(jnp.logical_not((tms <= TMAX) & (tms >= TMAX / 4)))
        def _():
            f = jnp.maximum(tm, TINY) * (1.0 / TMAX)
            fi = 1.0 / f

            def redo(sl, carry):
                r32 = pl.ds(pl.multiple_of(sl * 32, 32), 32)
                for g in range(4):
                    k_limbs(kt_s[r32, g * 128:(g + 1) * 128] * fi, g, r32)
                return carry
            jax.lax.fori_loop(0, S // 32, redo, 0)

            def resc(h, carry):
                sc_s[h] = sc_s[h] * f
                return carry
            jax.lax.fori_loop(0, H, resc, 0)

    def outproj(i, t, w):
        o = ot_s[:, rows(i * CPI + t)].T.astype(BF16)
        return x_s[t][i] + jnp.dot(o, unpacked(wo_s[w]), preferred_element_type=F32)

    def vt(h, cs):
        return unpacked(vt_s[pl.ds(pl.multiple_of(h * 8, 8), 8), cs])

    def finish(o, l, h, cs):
        lsum = jnp.sum(l, axis=0, keepdims=True)
        on = o * _recip(lsum)
        ot_s[pl.ds(pl.multiple_of(h * 16, 16), 16), cs] = on
        amax = jnp.maximum(jnp.abs(on[0:8]), jnp.abs(on[8:16]))
        lo, hi, om = stat_s[1], stat_s[2], stat_s[3]
        for t in range(on.shape[1] // 128):
            lt = lsum[:, t * 128:(t + 1) * 128]
            lo = jnp.minimum(lo, lt)
            hi = jnp.maximum(hi, lt)
            om = jnp.maximum(om, amax[:, t * 128:(t + 1) * 128])
        stat_s[1], stat_s[2], stat_s[3] = lo, hi, om

    def rev_slabs(n):
        return [t * 4 + j for t in range(n) for j in (3, 2, 1, 0)]

    def k_rev(h, k0, n):
        return jnp.concatenate([k8_s[h, k0 + r * 32:k0 + (r + 1) * 32, :] for r in rev_slabs(n)], axis=0)

    def unrev(p):
        return jnp.concatenate([p[r * 32:(r + 1) * 32] for r in rev_slabs(p.shape[0] // 128)], axis=0)

    def full_attention():
        nq = S // TQ
        nc = S // KC

        def body(i, carry):
            pend = []
            ls, os_ = {}, {}

            def do_pv():
                j, c, p, h, cs = pend.pop(0)
                co = jnp.dot(vt(h, slice(c * KC, (c + 1) * KC)), p, preferred_element_type=F32)
                os_[j] = co if j not in os_ else co + os_[j]
                if c == nc - 1:
                    finish(os_[j], ls[j], h, cs)

            for j in range(NSUB):
                u = NSUB * i + j
                h = u // nq
                cs = pl.ds(pl.multiple_of((u % nq) * TQ, TQ), TQ)
                sc = sc_s[h, 0:1, cs]
                for c in range(nc):
                    s = jnp.dot(k_rev(h, c * KC, KC // 128), q8_s[h, :, cs], preferred_element_type=I32)
                    p = jnp.exp2(s.astype(F32) * sc)
                    ls[j] = colacc(jnp.add, ls.get(j), p)
                    pend.append((j, c, unrev(p).astype(BF16), h, cs))
                    if len(pend) > 1:
                        do_pv()
            while pend:
                do_pv()
            return carry
        jax.lax.fori_loop(0, H * nq // NSUB, body, 0)

    def window_attention():
        def blk(b):
            return slice(b * 128, (b + 1) * 128)

        def body(it, carry):
            low = unrev(jax.lax.broadcasted_iota(I32, (128, 128), 0)) <= jax.lax.broadcasted_iota(I32, (128, 128), 1)
            pairs = [(j, i, 'd') for i in range(2, NB) for j in range(NHW)]
            single = [(j, i, 'd') for i in range(2) for j in range(NHW)] + \
                     [(j, i, 'm') for i in range(1, NB) for j in range(NHW)]
            rounds = []
            while pairs or single:
                if single and (not pairs or single[0][1] <= pairs[0][1]):
                    rounds.append(single[:4])
                    single = single[4:]
                else:
                    rounds.append(pairs[:2])
                    pairs = pairs[2:]
            rounds = [sum(rounds[r:r + RG], []) for r in range(0, len(rounds), RG)]
            unit = {(j, i): {'l': None, 'o': None, 'left': min(i, 2) + 1} for j in range(NHW) for i in range(NB)}
            pend = []

            def do_pv(tiles):
                for (j, i, kb, p) in tiles:
                    h = it * NHW + j
                    a = unit[(j, i)]
                    co = jnp.dot(vt(h, blk(kb)), p, preferred_element_type=F32)
                    a['o'] = co if a['o'] is None else co + a['o']
                    a['left'] -= 1
                    if a['left'] == 0:
                        finish(a['o'], a['l'], h, blk(i))

            for rnd in rounds:
                ss = []
                for (j, i, kind) in rnd:
                    h = it * NHW + j

                    def qk(kb):
                        return jnp.dot(k_rev(h, kb * 128, 1), q8_s[h, :, blk(i)], preferred_element_type=I32)
                    if kind == 'm':
                        ss.append(qk(i - 1))
                    elif i < 2:
                        ss.append(qk(i))
                    else:
                        ss.append(jnp.where(low, qk(i), qk(i - 2)))
                tiles = []
                for (j, i, kind), s in zip(rnd, ss):
                    p = jnp.exp2(s.astype(F32) * sc_s[it * NHW + j, 0:1, blk(i)])
                    if kind == 'd' and i < 2:
                        p = jnp.where(low, p, 0.0)
                    a = unit[(j, i)]
                    a['l'] = colacc(jnp.add, a['l'], p)
                    if kind == 'm':
                        tiles.append((j, i, i - 1, unrev(p).astype(BF16)))
                    elif i < 2:
                        tiles.append((j, i, i, unrev(p).astype(BF16)))
                    else:
                        tiles.append((j, i, i, unrev(jnp.where(low, p, 0.0)).astype(BF16)))
                        tiles.append((j, i, i - 2, unrev(jnp.where(low, 0.0, p)).astype(BF16)))
                pend.append(tiles)
                if len(pend) > WLAG:
                    do_pv(pend.pop(0))
            while pend:
                do_pv(pend.pop(0))
            return carry
        jax.lax.fori_loop(0, H // NHW, body, 0)

    def safe_attention(lo, hi):
        nq = S // TQ
        dq = (jax.lax.broadcasted_iota(I32, (128, TQ), 1) - jax.lax.broadcasted_iota(I32, (128, TQ), 0))

        def unit(u, carry):
            h = u // nq
            q0 = (u % nq) * TQ
            cs = pl.ds(pl.multiple_of(q0, TQ), TQ)
            sc = sc_s[h, 0:1, cs]

            def pass_a(c, m):
                kr = pl.ds(pl.multiple_of(c * 128, 128), 128)
                s = jnp.dot(k8_s[h, kr, :], q8_s[h, :, cs], preferred_element_type=I32)
                rel = dq + (q0 - c * 128)
                x = jnp.where((rel >= lo) & (rel < hi), s.astype(F32) * sc, NEG)
                sf_s[kr, :] = x
                return colacc(jnp.maximum, m, x)
            m = jax.lax.fori_loop(0, NB, pass_a, jnp.full((8, TQ), NEG, F32))
            m = jnp.max(m, axis=0, keepdims=True)

            def pass_b(c, lo_):
                l, o = lo_
                kr = pl.ds(pl.multiple_of(c * 128, 128), 128)
                p = jnp.exp2(sf_s[kr, :] - m)
                l = colacc(jnp.add, l, p)
                o = o + jnp.dot(vt(h, kr), p.astype(BF16), preferred_element_type=F32)
                return l, o
            l, o = jax.lax.fori_loop(0, NB, pass_b, (jnp.zeros((8, TQ), F32), jnp.zeros((16, TQ), F32)))
            ot_s[pl.ds(pl.multiple_of(h * 16, 16), 16), cs] = o / jnp.sum(l, axis=0, keepdims=True)
            return carry
        jax.lax.fori_loop(0, H * nq, unit, 0)

    stat_s[0] = jnp.zeros((8, 128), F32)
    with jax.named_scope("waitA"):
        w_copies[0].wait()
    with jax.named_scope("prepA"):
        prep_qkv(0)

    def first(i, carry):
        x_copy(i).wait()
        for t in range(CPI):
            x = xio_s[rows(i * CPI + t), :].astype(F32)
            x_s[t][i] = x
            xn_s[t][i] = packed(layernorm(x))
        project(i, 0)
        return carry
    with jax.named_scope("first"):
        jax.lax.fori_loop(0, NX, first, 0)

    with jax.named_scope("prepB"):
        for cp in w_copies[1:]:
            cp.wait()
        prep_qkv(1)
        for w in range(2):
            wo_s[w] = packed(woraw_s[w])

    def layer(l, carry):
        w = l % 2
        check_k_range()

        @pl.when(w == 0)
        def _():
            with jax.named_scope("window"):
                window_attention()

        @pl.when(w == 1)
        def _():
            with jax.named_scope("full"):
                full_attention()

        ok = (stat_s[1] > L_LO) & (stat_s[2] < L_HI) & (stat_s[3] < O_HI)

        @pl.when(jnp.max(jnp.where(ok, 0.0, 1.0)) > 0.0)
        def _():
            safe_attention(jnp.where(w == 0, 0, -S), jnp.where(w == 0, WIN, S))

        @pl.when(l < 3)
        def _():
            def mid(i, carry):
                for t in range(CPI):
                    x = outproj(i, t, w)
                    x_s[t][i] = x
                    xn_s[t][i] = packed(layernorm(x))
                project(i, 1 - w)
                return carry
            with jax.named_scope("mid"):
                jax.lax.fori_loop(0, NX, mid, 0)
        return carry
    jax.lax.fori_loop(0, 4, layer, 0)

    def last(i, carry):
        for t in range(CPI):
            xio_s[rows(i * CPI + t), :] = outproj(i, t, 1).astype(BF16)
        out_copy(i).start()
        return carry
    with jax.named_scope("last"):
        jax.lax.fori_loop(0, NX, last, 0)
    with jax.named_scope("outwait"):
        for i in range(NX):
            out_copy(i).wait()


@jax.jit
def pallas_interleave_layers__sliding_block__mha_block__prompt_kernel(A_x, A_wqkv, A_wo, B_x, B_wqkv, B_wo):
    del B_x
    out = pl.pallas_call(
        _kernel,
        out_shape=jax.ShapeDtypeStruct((S, D), BF16),
        in_specs=[pl.BlockSpec(memory_space=pl.ANY)] * 5,
        out_specs=pl.BlockSpec(memory_space=pl.ANY),
        scratch_shapes=[
            pltpu.VMEM((S, D), BF16),
            pltpu.VMEM((2, D, 3 * D), BF16),
            pltpu.VMEM((2, D, D), BF16),
            pltpu.VMEM((2, D // 2, D), U32),
            pltpu.VMEM((2, D, D), U32),
            pltpu.VMEM((2, D // 2, D), U32),
            pltpu.VMEM((2, 8, D), F32),
            pltpu.VMEM((2, D, 128), F32),
            pltpu.VMEM((S, D), F32),
            pltpu.VMEM((H, S, 128), I8),
            pltpu.VMEM((H, 128, S), I8),
            pltpu.VMEM((H, 8, S), F32),
            pltpu.VMEM((D // 2, S), U32),
            pltpu.VMEM((D, S), F32),
            pltpu.VMEM((2, 128, 128), I32),
            pltpu.VMEM((4, 8, 128), F32),
            pltpu.VMEM((S, TQ), F32),
            pltpu.SemaphoreType.DMA((4 + NX,)),
        ] + [pltpu.VMEM((NX, RC, D), F32)] * CPI
          + [pltpu.VMEM((NX, RC // 2, D), U32)] * CPI,
        compiler_params=pltpu.CompilerParams(vmem_limit_bytes=110 * 1024 * 1024),
        name="fused4",
    )(A_x.reshape(S, D), A_wqkv, A_wo, B_wqkv, B_wo)
    return out.reshape(1, S, D)
```

```python
import math

import jax
import jax.numpy as jnp
import jax.experimental.pallas as pl
import jax.experimental.pallas.tpu as pltpu

S, D, H, DH, WIN = 2048, 512, 32, 16, 256
F32, BF16, I32, I8, U32 = jnp.float32, jnp.bfloat16, jnp.int32, jnp.int8, jnp.uint32
QSCALE = (DH ** -0.5) * math.log2(math.e)
NEG = -1e30
RC = 256
NRC = S // RC
NX = NRC // 2
TQ = 512
KC = 256
NSUB = 16
NHW = 16
NB = S // 128
PVORD = '36047125'
WMODE = 0
NT = (((1,), (1,)), ((), ()))
FRAC = 64.0
TMAX = 127.0 * FRAC
MAGIC = 12582912.0
TINY = 1e-30
RK = 6.5
L_LO, L_HI, V_HI = 2.0 ** -60, 2.0 ** 60, 2.0 ** 60
WQ_A, WQ_B, WV_B, WO_A, WO_B, WV_A = range(6)
ST_K, ST_LMIN, ST_LMAX, ST_V, ST_ZERO, ST_VACC = range(6)


def _recip(x):
    r = pl.reciprocal(x, approx=True)
    return r * (2.0 - x * r)


def _limbs(t):
    u32 = pltpu.bitcast(t + (MAGIC + 32.0), I32)
    h = u32 >> 6
    bl = u32 & 63
    b = bl - 32
    d = (bl - 28) >> 3
    u512 = u32 + 480
    a = u512 >> 10
    c = ((u512 & 1023) - 448) >> 7
    return h, a, b, c, d


def _colacc(op, m, s):
    for i in range(s.shape[0] // 8):
        x = s[i * 8:(i + 1) * 8]
        m = x if m is None else op(m, x)
    return m


def _layernorm(x):
    mu = jnp.mean(x, axis=-1, keepdims=True)
    xc = x - mu
    var = jnp.mean(xc * xc, axis=-1, keepdims=True)
    return (xc * jax.lax.rsqrt(var + 1e-5)).astype(BF16)


def _packed(v):
    return pltpu.bitcast(v, U32)


def _unpacked(v):
    return pltpu.bitcast(v, BF16)


def _transposed(w):
    return _packed(w.astype(F32).T.astype(BF16))


def _unrev(p):
    return jnp.concatenate([p[t * 128 + r * 8:t * 128 + (r + 1) * 8]
                            for t in range(p.shape[0] // 128) for r in range(15, -1, -1)], axis=0)


def _kernel(x_hbm, wa_hbm, woa_hbm, wb_hbm, wob_hbm, out_hbm,
            xio_s, raw_s, wk_s, wt_s, wva_s, kinv_s, acol_s, kt_s, k8_s, q8_s, sc_s, vt_s, ot_s,
            stat_s, sf_s, pc_s, oc_s, lc_s, flag_s, sems, xa_s, xb_s, xna_s, xnb_s):
    x_s = (xa_s, xb_s)
    xn_s = (xna_s, xnb_s)

    def rows(c):
        return pl.ds(pl.multiple_of(c * RC, RC), RC)

    def cols(c, n):
        return pl.ds(pl.multiple_of(c * RC + n * 128, 128), 128)

    def hrows(h):
        return pl.ds(pl.multiple_of(h * DH, DH), DH)

    def x_copy(c):
        return pltpu.make_async_copy(x_hbm.at[rows(c), :], xio_s.at[rows(c), :], sems.at[8 + c])

    def out_copy(c):
        return pltpu.make_async_copy(xio_s.at[rows(c), :], out_hbm.at[rows(c), :], sems.at[c])

    def wcol(src, j):
        return src.at[:, j * D:(j + 1) * D]

    def raw_copy(slot, src=woa_hbm):
        return pltpu.make_async_copy(src, raw_s.at[slot], sems.at[slot])

    def wk_copy(w, src=woa_hbm):
        return pltpu.make_async_copy(src, wk_s.at[w], sems.at[6 + w])

    wk_copy(0, wcol(wa_hbm, 1)).start()
    raw_copy(WV_A, wcol(wa_hbm, 2)).start()
    x_copy(0).start()
    raw_copy(WQ_A, wcol(wa_hbm, 0)).start()
    for c in range(1, 5):
        x_copy(c).start()
    raw_copy(WQ_B, wcol(wb_hbm, 0)).start()
    for c in range(5, NRC):
        x_copy(c).start()
    raw_copy(WV_B, wcol(wb_hbm, 2)).start()
    raw_copy(WO_A, woa_hbm).start()
    wk_copy(1, wcol(wb_hbm, 1)).start()
    raw_copy(WO_B, wob_hbm).start()

    def prep_alpha(w):
        for g in range(4):
            gl = slice(g * 128, (g + 1) * 128)
            wkf = wk_s[w, :, gl].astype(F32)
            alpha = jnp.maximum(jnp.sqrt(jnp.sum(wkf * wkf, axis=0, keepdims=True)), TINY)
            kinv_s[w, :, gl] = jnp.broadcast_to((TMAX / RK) / alpha, (8, 128))
            acol_s[w, gl, :] = jnp.broadcast_to(alpha * (QSCALE / TMAX), (128, 128)).T

    def xtile(i, t, n):
        return _unpacked(xn_s[t][i, n * 64:(n + 1) * 64, :])

    def k_limbs(t32, g, r32):
        lane_blk = jax.lax.broadcasted_iota(I32, (8, 128), 1) >> 4
        t32 = jnp.concatenate([t32[r * 8:(r + 1) * 8] for r in (3, 2, 1, 0)], axis=0)
        hk, ak, bk, ck, dk = [pltpu.bitcast(z.astype(I8), I32) for z in _limbs(t32)]
        kslots = (hk, hk, hk, hk, bk, ak, dk, ck)
        xs = [v if j == 0 else pltpu.roll(v, 16 * j, 1) for j, v in enumerate(kslots)]
        for s in range(3):
            bit = (lane_blk & (1 << s)) != 0
            xs = [jnp.where(bit, xs[(j + (1 << s)) % 8], xs[j]) for j in range(8)]
        for e in range(8):
            k8_s[g * 8 + e, r32, :] = pltpu.bitcast(xs[(-e) % 8], I8)

    def proj_k(i, t, w):
        c = 2 * i + t
        for g in range(4):
            gl = slice(g * 128, (g + 1) * 128)
            k = jnp.dot(_unpacked(xn_s[t][i]), wk_s[w, :, gl], preferred_element_type=F32)
            kt = k * kinv_s[w, 0:1, gl]
            kt_s[rows(c), gl] = kt
            stat_s[ST_K] = _colacc(jnp.maximum, stat_s[ST_K], jnp.abs(kt))
            for sl in range(RC // 32):
                k_limbs(kt[sl * 32:(sl + 1) * 32], g, pl.ds(pl.multiple_of(c * RC + sl * 32, 32), 32))

    def proj_v(i, t, wv):
        vs = []
        for n in range(RC // 128):
            v = jax.lax.dot_general(_unpacked(wv[...]), xtile(i, t, n), NT, preferred_element_type=F32)
            vt_s[:, cols(2 * i + t, n)] = v
            stat_s[ST_VACC] = _colacc(jnp.maximum, stat_s[ST_VACC], jnp.abs(v))
            vs.append(v)
        return jnp.concatenate(vs, axis=0)

    def proj_q(i, t, w):
        c = 2 * i + t
        for n in range(RC // 128):
            q = jax.lax.dot_general(_unpacked(wt_s[WQ_A + w]), xtile(i, t, n), NT, preferred_element_type=F32)
            q = (q * acol_s[w]).reshape(H, DH, 128)
            qm = jnp.maximum(jnp.max(jnp.abs(q), axis=1, keepdims=True), TINY)
            qi = pl.reciprocal(qm, approx=True)
            qm = qm * (2.0 - qm * qi)
            sc_s[:, :, cols(c, n)] = jnp.broadcast_to(qm * (RK * FRAC / (4.0 * 127.0)), (H, 8, 128))
            hq, aq, bq, cq, dq = _limbs(q * (qi * TMAX))
            qslots = (hq, hq, hq, hq, aq, bq, cq, dq)
            for h in range(H):
                blocks = [qslots[(beta - h) % 8][h] for beta in range(8)]
                q8_s[h, :, cols(c, n)] = jnp.concatenate(blocks, axis=0).astype(I8)

    def project(i, w, wv, between=None):
        proj_v(i, 0, wv)
        if between is not None:
            between()
        proj_k(i, 1, w)
        proj_q(i, 1, w)
        proj_k(i, 0, w)
        flag_s[0] = jnp.max(stat_s[ST_K])
        proj_q(i, 0, w)
        return proj_v(i, 1, wv)

    def check_k_range():
        tms = flag_s[0]
        stat_s[ST_K] = jnp.zeros((8, 128), F32)
        stat_s[ST_LMIN] = jnp.ones((8, 128), F32)
        stat_s[ST_LMAX] = jnp.ones((8, 128), F32)
        stat_s[ST_V] = stat_s[ST_VACC]
        stat_s[ST_VACC] = jnp.zeros((8, 128), F32)

        @pl.when(jnp.logical_not((tms <= TMAX) & (tms >= TMAX / 4)))
        def _():
            f = jnp.maximum(jnp.full((1, 128), tms, F32), TINY) * (1.0 / TMAX)
            fi = 1.0 / f

            def redo(sl, carry):
                r32 = pl.ds(pl.multiple_of(sl * 32, 32), 32)
                for g in range(4):
                    k_limbs(kt_s[r32, g * 128:(g + 1) * 128] * fi, g, r32)
                return carry
            jax.lax.fori_loop(0, S // 32, redo, 0)

            def resc(h, carry):
                sc_s[h] = sc_s[h] * f[:, 0:1]
                return carry
            jax.lax.fori_loop(0, H, resc, 0)

    def outproj_ln(i, t, w):
        for n in range(RC // 128):
            yt = jnp.dot(_unpacked(wt_s[WO_A + w]), ot_s[:, cols(2 * i + t, n)].astype(BF16),
                         preferred_element_type=F32)
            x = x_s[t][i, n * 128:(n + 1) * 128, :] + yt.T
            x_s[t][i, n * 128:(n + 1) * 128, :] = x
            xn_s[t][i, n * 64:(n + 1) * 64, :] = _packed(_layernorm(x))

    def k_rev(h, k0, n):
        order = [t * 4 + j for t in range(n) for j in (3, 2, 1, 0)]
        if isinstance(k0, int):
            return jnp.concatenate([k8_s[h, k0 + r * 32:k0 + (r + 1) * 32, :] for r in order], axis=0)
        return jnp.concatenate([k8_s[h, pl.ds(pl.multiple_of(k0 + r * 32, 32), 32), :] for r in order], axis=0)

    def finish(o, l, h, cs):
        lsum = jnp.sum(l, axis=0, keepdims=True)
        ot_s[hrows(h), cs] = o * _recip(lsum)
        lo, hi = stat_s[ST_LMIN], stat_s[ST_LMAX]
        for t in range(lsum.shape[1] // 128):
            lt = lsum[:, t * 128:(t + 1) * 128]
            lo = jnp.minimum(lo, lt)
            hi = jnp.maximum(hi, lt)
        stat_s[ST_LMIN], stat_s[ST_LMAX] = lo, hi

    def publish_check():
        ok = (stat_s[ST_LMIN] > L_LO) & (stat_s[ST_LMAX] < L_HI) & (stat_s[ST_V] < V_HI)
        flag_s[1] = jnp.max(jnp.where(ok, 0.0, 1.0))

    def full_attention():
        nq = S // TQ
        nc = S // KC

        def pv(h, c, p, o):
            o = [None] * 4 if o is None else [o[:, n * 128:(n + 1) * 128] for n in range(4)]
            for ch in PVORD:
                e, n = divmod(int(ch), 4)
                k0 = c * KC + e * 128
                co = jnp.dot(vt_s[hrows(h), k0:k0 + 128], p[e * 128:(e + 1) * 128, n * 128:(n + 1) * 128],
                             preferred_element_type=F32)
                o[n] = co if o[n] is None else co + o[n]
            return jnp.concatenate(o, axis=1)

        def carried(h):
            finish(pv(h, nc - 1, pc_s[...], oc_s[...]), lc_s[...], h, slice(S - TQ, S))

        def body(i, carry):
            pend = []
            ls, os_ = {}, {}
            for j in range(NSUB):
                h, cs = i * (NSUB // nq) + j // nq, slice((j % nq) * TQ, (j % nq + 1) * TQ)
                sc = sc_s[h, 0:1, cs]
                for c in range(nc):
                    s = jnp.dot(k_rev(h, c * KC, KC // 128), q8_s[h, :, cs], preferred_element_type=I32)
                    if j == 0 and c == 0:
                        carried(jnp.maximum(i * (NSUB // nq) - 1, 0))
                    p = jnp.exp2(s.astype(F32) * sc)
                    ls[j] = _colacc(jnp.add, ls.get(j), p)
                    pend.append((j, c, _unrev(p), h, cs))
                    if len(pend) > 1:
                        jp, cp, pp, hp, csp = pend.pop(0)
                        os_[jp] = pv(hp, cp, pp, os_.get(jp))
                        if cp == nc - 1:
                            finish(os_[jp], ls[jp], hp, csp)
            pc_s[...] = pend[0][2]
            oc_s[...] = os_[NSUB - 1]
            lc_s[...] = ls[NSUB - 1]
            return carry
        jax.lax.fori_loop(0, H * nq // NSUB, body, 0)
        carried(H - 1)
        publish_check()

    def window_attention():
        def blk(b):
            return slice(b * 128, (b + 1) * 128)

        def body(it, carry):
            pw = D * NHW // H
            wt_s[WO_B, pl.ds(pl.multiple_of(it * (pw // 2), pw // 2), pw // 2), :] = _transposed(
                raw_s[WO_B, :, pl.ds(pl.multiple_of(it * pw, pw), pw)])

            low = _unrev(jax.lax.broadcasted_iota(I32, (128, 128), 0)) <= jax.lax.broadcasted_iota(I32, (128, 128), 1)
            rounds = []
            for j0 in range(0, NHW, 8):
                js = range(j0, j0 + 8)
                pairs = [(j, i, 'd') for i in range(2, NB) for j in js]
                single = [(j, i, 'd') for i in range(2) for j in js] + [(j, i, 'm') for i in range(1, NB) for j in js]
                pr = [pairs[r:r + 2] for r in range(0, len(pairs), 2)]
                sr = [single[r:r + 4] for r in range(0, len(single), 4)]
                while pr or sr:
                    if sr and (len(pr) <= len(sr) or sr[0][0][1] <= pr[0][0][1] + (WMODE >> 1) - 1 + 1):
                        a, b = sr.pop(0), pr.pop(0)
                        rounds.append(b + a if WMODE & 1 else a + b)
                    else:
                        rounds.append(pr.pop(0) + pr.pop(0))
            unit = {(j, i): {'l': None, 'o': None, 'left': min(i, 2) + 1} for j in range(NHW) for i in range(NB)}
            pend = []

            def do_pv(tiles):
                for (j, i, kb, p) in tiles:
                    h = it * NHW + j
                    a = unit[(j, i)]
                    co = jnp.dot(vt_s[hrows(h), blk(kb)].astype(BF16), p.astype(BF16), preferred_element_type=F32)
                    a['o'] = co if a['o'] is None else co + a['o']
                    a['left'] -= 1
                    if a['left'] == 0:
                        finish(a['o'], a['l'], h, blk(i))

            def qk(j, i, kb):
                h = it * NHW + j
                return jnp.dot(k_rev(h, kb * 128, 1), q8_s[h, :, blk(i)], preferred_element_type=I32)

            for rnd in rounds:
                ss = []
                for (j, i, kind) in rnd:
                    if kind == 'm':
                        ss.append(qk(j, i, i - 1))
                    elif i < 2:
                        ss.append(qk(j, i, i))
                    else:
                        ss.append(jnp.where(low, qk(j, i, i), qk(j, i, i - 2)))
                tiles = []
                for (j, i, kind), s in zip(rnd, ss):
                    p = jnp.exp2(s.astype(F32) * sc_s[it * NHW + j, 0:1, blk(i)])
                    if kind == 'd' and i < 2:
                        p = jnp.where(low, p, 0.0)
                    a = unit[(j, i)]
                    a['l'] = _colacc(jnp.add, a['l'], p)
                    if kind == 'm':
                        tiles.append((j, i, i - 1, _unrev(p)))
                    elif i < 2:
                        tiles.append((j, i, i, _unrev(p)))
                    else:
                        tiles.append((j, i, i, _unrev(jnp.where(low, p, 0.0))))
                        tiles.append((j, i, i - 2, _unrev(jnp.where(low, 0.0, p))))
                pend.append(tiles)
                if len(pend) > 1:
                    do_pv(pend.pop(0))
            do_pv(pend.pop(0))
            publish_check()
            return carry
        jax.lax.fori_loop(0, H // NHW, body, 0)

    def safe_attention(lo, hi):
        nq = S // TQ
        dq = jax.lax.broadcasted_iota(I32, (128, TQ), 1) - jax.lax.broadcasted_iota(I32, (128, TQ), 0)

        def unit(u, carry):
            h = u // nq
            q0 = (u % nq) * TQ
            cs = pl.ds(pl.multiple_of(q0, TQ), TQ)
            sc = sc_s[h, 0:1, cs]

            def pass_a(c, m):
                s = _unrev(jnp.dot(k_rev(h, c * 128, 1), q8_s[h, :, cs], preferred_element_type=I32))
                rel = dq + (q0 - c * 128)
                x = jnp.where((rel >= lo) & (rel < hi), s.astype(F32) * sc, NEG)
                sf_s[pl.ds(pl.multiple_of(c * 128, 128), 128), :] = x
                return _colacc(jnp.maximum, m, x)
            m = jax.lax.fori_loop(0, NB, pass_a, jnp.full((8, TQ), NEG, F32))
            m = jnp.max(m, axis=0, keepdims=True)

            def pass_b(c, acc):
                l, o = acc
                kr = pl.ds(pl.multiple_of(c * 128, 128), 128)
                p = jnp.exp2(sf_s[kr, :] - m)
                l = _colacc(jnp.add, l, p)
                o = o + jnp.dot(vt_s[hrows(h), kr], p, preferred_element_type=F32)
                return l, o
            l, o = jax.lax.fori_loop(0, NB, pass_b, (jnp.zeros((8, TQ), F32), jnp.zeros((DH, TQ), F32)))
            ot_s[hrows(h), cs] = o / jnp.sum(l, axis=0, keepdims=True)
            return carry
        jax.lax.fori_loop(0, H * nq, unit, 0)

    def load_ln(i, t, pace=None):
        pr = RC if pace is None else 32
        for j in range(RC // pr):
            x = xio_s[pl.ds(pl.multiple_of((2 * i + t) * RC + j * pr, pr), pr), :].astype(F32)
            if pace is not None:
                r = j * 80
                z = pltpu.bitcast(pltpu.bitcast(pace[r:r + 8], I32) & pltpu.bitcast(stat_s[ST_ZERO], I32), F32)
                x = x + jnp.concatenate([z[0:1]] * 4, axis=1)
            x_s[t][i, j * pr:(j + 1) * pr, :] = x
            xn_s[t][i, j * pr // 2:(j + 1) * pr // 2, :] = _packed(_layernorm(x))

    stat_s[...] = jnp.zeros_like(stat_s)
    pc_s[...] = jnp.zeros_like(pc_s)
    oc_s[...] = jnp.zeros_like(oc_s)
    lc_s[...] = jnp.ones_like(lc_s)
    with jax.named_scope("prepA"):
        wk_copy(0).wait()
        prep_alpha(0)
        raw_copy(WV_A).wait()
        x_copy(0).wait()
        wv = _transposed(raw_s[WV_A])
        wva_s[...] = wv
        wt_s[WV_A] = wv
        load_ln(0, 0)

    def first(i, carry):
        raw_copy(i).wait()
        x_copy(2 * i + 1).wait()

        @pl.when(i + 1 < NX)
        def _():
            x_copy(2 * i + 2).wait()

        def prep():
            load_ln(i, 1)
            wt_s[i] = _transposed(raw_s[i])
        pace = project(i, 0, wva_s, prep)
        load_ln(jnp.minimum(i + 1, NX - 1), 0, pace)
        return carry
    with jax.named_scope("first"):
        jax.lax.fori_loop(0, NX, first, 0)
    raw_copy(WO_B).wait()
    wk_copy(1).wait()
    prep_alpha(1)

    def layer(l, carry):
        w = l % 2
        check_k_range()

        @pl.when(w == 0)
        def _():
            with jax.named_scope("window"):
                window_attention()

        @pl.when(w == 1)
        def _():
            with jax.named_scope("full"):
                full_attention()

        @pl.when(flag_s[1] > 0.0)
        def _():
            safe_attention(jnp.where(w == 0, 0, -S), jnp.where(w == 0, WIN, S))

        @pl.when(l < 3)
        def _():
            def mid(i, carry):
                outproj_ln(i, 0, w)
                outproj_ln(i, 1, w)
                project(i, 1 - w, wt_s.at[WV_B + 3 * w])
                return carry
            with jax.named_scope("mid"):
                jax.lax.fori_loop(0, NX, mid, 0)
        return carry
    jax.lax.fori_loop(0, 4, layer, 0)

    with jax.named_scope("last"):
        for c in range(NRC):
            o = ot_s[:, c * RC:(c + 1) * RC].T.astype(BF16)
            y = x_s[c % 2][c // 2] + jnp.dot(o, raw_s[WO_B], preferred_element_type=F32)
            xio_s[c * RC:(c + 1) * RC, :] = y.astype(BF16)
            out_copy(c).start()
    with jax.named_scope("outwait"):
        for c in range(NRC):
            out_copy(c).wait()


@jax.jit
def pallas_interleave_layers__sliding_block__mha_block__prompt_kernel(A_x, A_wqkv, A_wo, B_x, B_wqkv, B_wo):
    del B_x
    out = pl.pallas_call(
        _kernel,
        out_shape=jax.ShapeDtypeStruct((S, D), BF16),
        in_specs=[pl.BlockSpec(memory_space=pl.ANY)] * 5,
        out_specs=pl.BlockSpec(memory_space=pl.ANY),
        scratch_shapes=[
            pltpu.VMEM((S, D), BF16),
            pltpu.VMEM((6, D, D), BF16),
            pltpu.VMEM((2, D, D), BF16),
            pltpu.VMEM((6, D // 2, D), U32),
            pltpu.VMEM((D // 2, D), U32),
            pltpu.VMEM((2, 8, D), F32),
            pltpu.VMEM((2, D, 128), F32),
            pltpu.VMEM((S, D), F32),
            pltpu.VMEM((H, S, 128), I8),
            pltpu.VMEM((H, 128, S), I8),
            pltpu.VMEM((H, 8, S), F32),
            pltpu.VMEM((D, S), F32),
            pltpu.VMEM((D, S), F32),
            pltpu.VMEM((6, 8, 128), F32),
            pltpu.VMEM((S, TQ), F32),
            pltpu.VMEM((KC, TQ), F32),
            pltpu.VMEM((DH, TQ), F32),
            pltpu.VMEM((8, TQ), F32),
            pltpu.SMEM((2,), F32),
            pltpu.SemaphoreType.DMA((8 + NRC,)),
            pltpu.VMEM((NX, RC, D), F32),
            pltpu.VMEM((NX, RC, D), F32),
            pltpu.VMEM((NX, RC // 2, D), U32),
            pltpu.VMEM((NX, RC // 2, D), U32),
        ],
        compiler_params=pltpu.CompilerParams(vmem_limit_bytes=110 * 1024 * 1024),
        name="fused4",
    )(A_x.reshape(S, D), A_wqkv, A_wo, B_wqkv, B_wo)
    return out.reshape(1, S, D)
```

```python
import math

import jax
import jax.numpy as jnp
import jax.experimental.pallas as pl
import jax.experimental.pallas.tpu as pltpu

S, D, H, DH, WIN = 2048, 512, 32, 16, 256
F32, BF16, I32, I8, U32 = jnp.float32, jnp.bfloat16, jnp.int32, jnp.int8, jnp.uint32
QSCALE = (DH ** -0.5) * math.log2(math.e)
MASKED = -1e9 * math.log2(math.e)
RC = 256
NRC = S // RC
NX = NRC // 2
TQ = 512
KC = 256
NSUB = 16
NHW = 16
NB = S // 128
PVORD = (3, 6, 0, 4, 7, 1, 2, 5)
WPERM = (0, 1, 3, 7, 6, 4, 5, 2)
NT = (((1,), (1,)), ((), ()))
FRAC = 64.0
TMAX = 127.0 * FRAC
QMAX = 126.0 * FRAC
MAGIC = 12582912.0
TINY = 1e-30
RK = 6.5
L_LO, L_HI, V_HI = 2.0 ** -60, 2.0 ** 60, 2.0 ** 60
WQ_A, WQ_B, WV_B, WO_A, WO_B, WV_A = range(6)
ST_K, ST_LMIN, ST_LMAX, ST_V, ST_ZERO, ST_VACC = range(6)


def _recip(x):
    r = pl.reciprocal(x, approx=True)
    return r * (2.0 - x * r)


def _limbs(t):
    u32 = pltpu.bitcast(t + (MAGIC + 32.0), I32)
    h = u32 >> 6
    bl = u32 & 63
    b = bl - 32
    d = (bl - 28) >> 3
    u512 = u32 + 480
    a = u512 >> 10
    c = ((u512 & 1023) - 448) >> 7
    return h, a, b, c, d


def _colacc(op, m, s):
    for i in range(s.shape[0] // 8):
        x = s[i * 8:(i + 1) * 8]
        m = x if m is None else op(m, x)
    return m


def _layernorm(x):
    mu = jnp.mean(x, axis=-1, keepdims=True)
    xc = x - mu
    var = jnp.mean(xc * xc, axis=-1, keepdims=True)
    return (xc * jax.lax.rsqrt(var + 1e-5)).astype(BF16)


def _packed(v):
    return pltpu.bitcast(v, U32)


def _unpacked(v):
    return pltpu.bitcast(v, BF16)


def _transposed(w):
    return _packed(w.astype(F32).T.astype(BF16))


def _unrev(p):
    return jnp.concatenate([p[t * 128 + r * 8:t * 128 + (r + 1) * 8]
                            for t in range(p.shape[0] // 128) for r in range(15, -1, -1)], axis=0)


def _kernel(x_hbm, wa_hbm, woa_hbm, wb_hbm, wob_hbm, out_hbm,
            xio_s, raw_s, wk_s, wt_s, wva_s, kinv_s, acol_s, kt_s, k8_s, q8_s, sc_s, vt_s, ot_s,
            stat_s, sf_s, pc_s, oc_s, lc_s, flag_s, sems, xa_s, xb_s, xna_s, xnb_s):
    x_s = (xa_s, xb_s)
    xn_s = (xna_s, xnb_s)

    def rows(c):
        return pl.ds(pl.multiple_of(c * RC, RC), RC)

    def span(i, off, size):
        return pl.ds(pl.multiple_of(i * (2 * RC), 2 * RC) + off, size)

    def cols(i, t, n):
        return span(i, t * RC + n * 128, 128)

    def hrows(h):
        return pl.ds(pl.multiple_of(h * DH, DH), DH)

    def x_copy(c):
        return pltpu.make_async_copy(x_hbm.at[rows(c), :], xio_s.at[rows(c), :], sems.at[8 + c])

    def wcol(src, j):
        return src.at[:, j * D:(j + 1) * D]

    def raw_copy(slot, src=woa_hbm):
        return pltpu.make_async_copy(src, raw_s.at[slot], sems.at[slot])

    def wk_copy(w, src=woa_hbm):
        return pltpu.make_async_copy(src, wk_s.at[w], sems.at[6 + w])

    wk_copy(0, wcol(wa_hbm, 1)).start()
    raw_copy(WV_A, wcol(wa_hbm, 2)).start()
    x_copy(0).start()
    raw_copy(WQ_A, wcol(wa_hbm, 0)).start()
    for c in range(1, 5):
        x_copy(c).start()
    raw_copy(WQ_B, wcol(wb_hbm, 0)).start()
    for c in range(5, NRC):
        x_copy(c).start()
    raw_copy(WV_B, wcol(wb_hbm, 2)).start()
    raw_copy(WO_A, woa_hbm).start()
    wk_copy(1, wcol(wb_hbm, 1)).start()
    raw_copy(WO_B, wob_hbm).start()

    def prep_alpha(w):
        wkf = wk_s[w].astype(F32)
        sq = wkf * wkf
        sq = sq[0:256] + sq[256:512]
        sq = sq[0:128] + sq[128:256]
        ss = jnp.maximum(jnp.sum(sq, axis=0, keepdims=True), TINY)
        r = jax.lax.rsqrt(ss)
        kinv_s[w] = jnp.broadcast_to(r * (TMAX / RK), (8, D))
        acol_s[w] = jnp.broadcast_to((ss * r) * (QSCALE / TMAX), (128, D)).T

    def xtile(i, t, n):
        return _unpacked(xn_s[t][i, n * 64:(n + 1) * 64, :])

    def k_limbs(t32, g, r32):
        lane_blk = jax.lax.broadcasted_iota(I32, (8, 128), 1) >> 4
        t32 = jnp.concatenate([t32[r * 8:(r + 1) * 8] for r in (3, 2, 1, 0)], axis=0)
        hk, ak, bk, ck, dk = [pltpu.bitcast(z.astype(I8), I32) for z in _limbs(t32)]
        kslots = (hk, hk, hk, hk, bk, ak, dk, ck)
        xs = [v if j == 0 else pltpu.roll(v, 16 * j, 1) for j, v in enumerate(kslots)]
        for s in range(3):
            bit = (lane_blk & (1 << s)) != 0
            xs = [jnp.where(bit, xs[(j + (1 << s)) % 8], xs[j]) for j in range(8)]
        for e in range(8):
            k8_s[g * 8 + e, r32, :] = pltpu.bitcast(xs[(-e) % 8], I8)

    def proj_k(i, t, w):
        for g in range(4):
            gl = slice(g * 128, (g + 1) * 128)
            k = jnp.dot(_unpacked(xn_s[t][i]), wk_s[w, :, gl], preferred_element_type=F32)
            kt = k * kinv_s[w, 0:1, gl]
            kt_s[span(i, t * RC, RC), gl] = kt
            stat_s[ST_K] = _colacc(jnp.maximum, stat_s[ST_K], jnp.abs(kt))
            for sl in range(RC // 32):
                k_limbs(kt[sl * 32:(sl + 1) * 32], g, span(i, t * RC + sl * 32, 32))

    def proj_v(i, t, wv):
        vs = []
        for n in range(RC // 128):
            v = jax.lax.dot_general(_unpacked(wv[...]), xtile(i, t, n), NT, preferred_element_type=F32)
            vt_s[:, cols(i, t, n)] = v
            stat_s[ST_VACC] = _colacc(jnp.maximum, stat_s[ST_VACC], jnp.abs(v))
            vs.append(v)
        return jnp.concatenate(vs, axis=0)

    def proj_q(i, t, w):
        for n in range(RC // 128):
            q = jax.lax.dot_general(_unpacked(wt_s[WQ_A + w]), xtile(i, t, n), NT, preferred_element_type=F32)
            q = (q * acol_s[w]).reshape(H, DH, 128)
            qm = jnp.maximum(jnp.max(jnp.abs(q), axis=1, keepdims=True), TINY)
            qi = pl.reciprocal(qm, approx=True)
            qm = qm * (2.0 - qm * qi)
            sc_s[:, :, cols(i, t, n)] = jnp.broadcast_to(qm * (RK * 1024.0 / QMAX), (H, 8, 128))
            hq, aq, bq, cq, dq = _limbs(q * (qi * QMAX))
            qslots = (hq, hq, hq, hq, aq, bq, cq, dq)
            for h in range(H):
                blocks = [qslots[(beta - h) % 8][h] for beta in range(8)]
                q8_s[h, :, cols(i, t, n)] = jnp.concatenate(blocks, axis=0).astype(I8)

    def project(i, w, wv, between=None):
        proj_v(i, 0, wv)
        if between is not None:
            between()
        proj_k(i, 1, w)
        proj_q(i, 1, w)
        proj_k(i, 0, w)
        flag_s[0] = jnp.max(stat_s[ST_K])
        proj_q(i, 0, w)
        return proj_v(i, 1, wv)

    def check_k_range():
        tms = flag_s[0]
        stat_s[ST_K] = jnp.zeros((8, 128), F32)
        stat_s[ST_LMIN] = jnp.ones((8, 128), F32)
        stat_s[ST_LMAX] = jnp.ones((8, 128), F32)
        stat_s[ST_V] = stat_s[ST_VACC]
        stat_s[ST_VACC] = jnp.zeros((8, 128), F32)

        @pl.when(jnp.logical_not((tms <= TMAX) & (tms >= TMAX / 4)))
        def _():
            f = jnp.maximum(jnp.full((1, 128), tms, F32), TINY) * (1.0 / TMAX)
            fi = 1.0 / f

            def redo(sl, carry):
                r32 = pl.ds(pl.multiple_of(sl * 32, 32), 32)
                for g in range(4):
                    k_limbs(kt_s[r32, g * 128:(g + 1) * 128] * fi, g, r32)
                return carry
            jax.lax.fori_loop(0, S // 32, redo, 0)

            def resc(h, carry):
                sc_s[h] = sc_s[h] * f[:, 0:1]
                return carry
            jax.lax.fori_loop(0, H, resc, 0)

    def outproj_ln(i, t, w):
        for n in range(RC // 128):
            yt = jnp.dot(_unpacked(wt_s[WO_A + w]), ot_s[:, cols(i, t, n)].astype(BF16),
                         preferred_element_type=F32)
            x = x_s[t][i, n * 128:(n + 1) * 128, :] + yt.T
            x_s[t][i, n * 128:(n + 1) * 128, :] = x
            xn_s[t][i, n * 64:(n + 1) * 64, :] = _packed(_layernorm(x))

    def k_rev(h, k0, n):
        order = [t * 4 + j for t in range(n) for j in (3, 2, 1, 0)]
        if isinstance(k0, int):
            return jnp.concatenate([k8_s[h, k0 + r * 32:k0 + (r + 1) * 32, :] for r in order], axis=0)
        return jnp.concatenate([k8_s[h, pl.ds(pl.multiple_of(k0 + r * 32, 32), 32), :] for r in order], axis=0)

    def finish(o, l, h, cs):
        lsum = jnp.sum(l, axis=0, keepdims=True)
        ot_s[hrows(h), cs] = o * _recip(lsum)
        lo, hi = stat_s[ST_LMIN], stat_s[ST_LMAX]
        for t in range(lsum.shape[1] // 128):
            lt = lsum[:, t * 128:(t + 1) * 128]
            lo = jnp.minimum(lo, lt)
            hi = jnp.maximum(hi, lt)
        stat_s[ST_LMIN], stat_s[ST_LMAX] = lo, hi

    def publish_check():
        ok = (stat_s[ST_LMIN] > L_LO) & (stat_s[ST_LMAX] < L_HI) & (stat_s[ST_V] < V_HI)
        flag_s[1] = jnp.max(jnp.where(ok, 0.0, 1.0))

    def full_attention():
        nq = S // TQ
        nc = S // KC

        def pv(h, c, p, o):
            o = [None] * 4 if o is None else [o[:, n * 128:(n + 1) * 128] for n in range(4)]
            for tile in PVORD:
                e, n = divmod(tile, 4)
                k0 = c * KC + e * 128
                co = jnp.dot(vt_s[hrows(h), k0:k0 + 128], p[e * 128:(e + 1) * 128, n * 128:(n + 1) * 128],
                             preferred_element_type=F32)
                o[n] = co if o[n] is None else co + o[n]
            return jnp.concatenate(o, axis=1)

        def carried(h):
            finish(pv(h, nc - 1, pc_s[...], oc_s[...]), lc_s[...], h, slice(S - TQ, S))

        def body(i, carry):
            pend = []
            ls, os_ = {}, {}
            for j in range(NSUB):
                h, cs = i * (NSUB // nq) + j // nq, slice((j % nq) * TQ, (j % nq + 1) * TQ)
                sc = sc_s[h, 0:1, cs]
                for c in range(nc):
                    s = jnp.dot(k_rev(h, c * KC, KC // 128), q8_s[h, :, cs], preferred_element_type=I32)
                    if j == 0 and c == 0:
                        carried(jnp.maximum(i * (NSUB // nq) - 1, 0))
                    p = jnp.exp2(s.astype(F32) * sc)
                    ls[j] = _colacc(jnp.add, ls.get(j), p)
                    pend.append((j, c, _unrev(p), h, cs))
                    if len(pend) > 1:
                        jp, cp, pp, hp, csp = pend.pop(0)
                        os_[jp] = pv(hp, cp, pp, os_.get(jp))
                        if cp == nc - 1:
                            finish(os_[jp], ls[jp], hp, csp)
            pc_s[...] = pend[0][2]
            oc_s[...] = os_[NSUB - 1]
            lc_s[...] = ls[NSUB - 1]
            return carry
        jax.lax.fori_loop(0, H * nq // NSUB, body, 0)
        carried(H - 1)
        publish_check()

    def window_attention():
        def blk(b):
            return slice(b * 128, (b + 1) * 128)

        def body(it, carry):
            pw = D * NHW // H
            wt_s[WO_B, pl.ds(pl.multiple_of(it * (pw // 2), pw // 2), pw // 2), :] = _transposed(
                raw_s[WO_B, :, pl.ds(pl.multiple_of(it * pw, pw), pw)])

            low = _unrev(jax.lax.broadcasted_iota(I32, (128, 128), 0)) <= jax.lax.broadcasted_iota(I32, (128, 128), 1)
            rounds = []
            for j0 in range(0, NHW, 8):
                js = range(j0, j0 + 8)
                pairs = [(j, i, 'd') for i in range(2, NB) for j in js]
                single = [(j, i, 'd') for i in range(2) for j in js] + [(j, i, 'm') for i in range(1, NB) for j in js]
                pr = [pairs[r:r + 2] for r in range(0, len(pairs), 2)]
                sr = [single[r:r + 4] for r in range(0, len(single), 4)]
                while pr or sr:
                    if sr and (len(pr) <= len(sr) or sr[0][0][1] <= pr[0][0][1]):
                        rounds.append(sr.pop(0) + pr.pop(0))
                    else:
                        rounds.append(pr.pop(0) + pr.pop(0))
            unit = {(j, i): {'l': None, 'o': None, 'left': min(i, 2) + 1} for j in range(NHW) for i in range(NB)}
            pend = []

            def do_pv(tiles):
                for (j, i, kb, p) in tiles:
                    h = it * NHW + j
                    a = unit[(j, i)]
                    co = jnp.dot(vt_s[hrows(h), blk(kb)].astype(BF16), p.astype(BF16), preferred_element_type=F32)
                    a['o'] = co if a['o'] is None else co + a['o']
                    a['left'] -= 1
                    if a['left'] == 0:
                        finish(a['o'], a['l'], h, blk(i))

            def qk(j, i, kb):
                h = it * NHW + j
                return jnp.dot(k_rev(h, kb * 128, 1), q8_s[h, :, blk(i)], preferred_element_type=I32)

            for rnd in rounds:
                ss = []
                for (j, i, kind) in rnd:
                    if kind == 'm':
                        ss.append(qk(j, i, i - 1))
                    elif i < 2:
                        ss.append(qk(j, i, i))
                    else:
                        ss.append(jnp.where(low, qk(j, i, i), qk(j, i, i - 2)))
                tiles = []
                for (j, i, kind), s in zip(rnd, ss):
                    p = jnp.exp2(s.astype(F32) * sc_s[it * NHW + j, 0:1, blk(i)])
                    if kind == 'd' and i < 2:
                        p = jnp.where(low, p, 0.0)
                    a = unit[(j, i)]
                    a['l'] = _colacc(jnp.add, a['l'], p)
                    if kind == 'm':
                        tiles.append((j, i, i - 1, _unrev(p)))
                    elif i < 2:
                        tiles.append((j, i, i, _unrev(p)))
                    else:
                        tiles.append((j, i, i, _unrev(jnp.where(low, p, 0.0))))
                        tiles.append((j, i, i - 2, _unrev(jnp.where(low, 0.0, p))))
                pend.append([tiles[e] for e in WPERM])
                if len(pend) > 1:
                    do_pv(pend.pop(0))
            do_pv(pend.pop(0))
            publish_check()
            return carry
        jax.lax.fori_loop(0, H // NHW, body, 0)

    def safe_attention(lo, hi):
        nq = S // TQ
        dq = jax.lax.broadcasted_iota(I32, (128, TQ), 1) - jax.lax.broadcasted_iota(I32, (128, TQ), 0)

        def unit(u, carry):
            h = u // nq
            q0 = (u % nq) * TQ
            cs = pl.ds(pl.multiple_of(q0, TQ), TQ)
            sc = sc_s[h, 0:1, cs]

            def pass_a(c, m):
                s = _unrev(jnp.dot(k_rev(h, c * 128, 1), q8_s[h, :, cs], preferred_element_type=I32))
                rel = dq + (q0 - c * 128)
                x = jnp.where((rel >= lo) & (rel < hi), s.astype(F32) * sc, MASKED)
                sf_s[pl.ds(pl.multiple_of(c * 128, 128), 128), :] = x
                return _colacc(jnp.maximum, m, x)
            m = jax.lax.fori_loop(0, NB, pass_a, jnp.full((8, TQ), -jnp.inf, F32))
            m = jnp.max(m, axis=0, keepdims=True)

            def pass_b(c, acc):
                l, o = acc
                kr = pl.ds(pl.multiple_of(c * 128, 128), 128)
                p = jnp.exp2(sf_s[kr, :] - m)
                l = _colacc(jnp.add, l, p)
                o = o + jnp.dot(vt_s[hrows(h), kr], p, preferred_element_type=F32)
                return l, o
            l, o = jax.lax.fori_loop(0, NB, pass_b, (jnp.zeros((8, TQ), F32), jnp.zeros((DH, TQ), F32)))
            ot_s[hrows(h), cs] = o / jnp.sum(l, axis=0, keepdims=True)
            return carry
        jax.lax.fori_loop(0, H * nq, unit, 0)

    def load_ln(i, t, pace=None):
        pr = RC if pace is None else 32
        for j in range(RC // pr):
            x = xio_s[span(i, t * RC + j * pr, pr), :].astype(F32)
            if pace is not None:
                r = j * 80
                z = pltpu.bitcast(pltpu.bitcast(pace[r:r + 8], I32) & pltpu.bitcast(stat_s[ST_ZERO], I32), F32)
                x = x + jnp.concatenate([z[0:1]] * 4, axis=1)
            x_s[t][i, j * pr:(j + 1) * pr, :] = x
            xn_s[t][i, j * pr // 2:(j + 1) * pr // 2, :] = _packed(_layernorm(x))

    flag_s[0] = 0.0
    flag_s[1] = 0.0
    stat_s[...] = jnp.zeros_like(stat_s)
    pc_s[...] = jnp.zeros_like(pc_s)
    oc_s[...] = jnp.zeros_like(oc_s)
    lc_s[...] = jnp.ones_like(lc_s)
    wk_copy(0).wait()
    prep_alpha(0)
    raw_copy(WV_A).wait()
    x_copy(0).wait()
    wv = _transposed(raw_s[WV_A])
    wva_s[...] = wv
    wt_s[WV_A] = wv
    load_ln(0, 0)

    def first(i, carry):
        raw_copy(i).wait()
        x_copy(2 * i + 1).wait()

        @pl.when(i + 1 < NX)
        def _():
            x_copy(2 * i + 2).wait()

        def prep():
            load_ln(i, 1)
            wt_s[i] = _transposed(raw_s[i])
        pace = project(i, 0, wva_s, prep)
        load_ln(jnp.minimum(i + 1, NX - 1), 0, pace)
        return carry
    jax.lax.fori_loop(0, NX, first, 0)
    raw_copy(WO_B).wait()
    wk_copy(1).wait()
    prep_alpha(1)

    def layer(l, carry):
        w = l % 2
        check_k_range()

        @pl.when(w == 0)
        def _():
            window_attention()

        @pl.when(w == 1)
        def _():
            full_attention()

        @pl.when(flag_s[1] > 0.0)
        def _():
            safe_attention(jnp.where(w == 0, 0, -S), jnp.where(w == 0, WIN, S))

        @pl.when(l < 3)
        def _():
            def mid(i, carry):
                outproj_ln(i, 0, w)
                outproj_ln(i, 1, w)
                project(i, 1 - w, wt_s.at[WV_B + 3 * w])
                return carry
            jax.lax.fori_loop(0, NX, mid, 0)
        return carry
    jax.lax.fori_loop(0, 4, layer, 0)

    pieces = [(0, 128), (128, 128)] + [(c * RC, RC) for c in range(1, NRC - 1)] + [(S - RC, 128), (S - 128, 128)]

    def out_copy(k):
        r0, n = pieces[k]
        return pltpu.make_async_copy(xio_s.at[r0:r0 + n, :], out_hbm.at[r0:r0 + n, :], sems.at[k])

    for k, (r0, n) in enumerate(pieces):
        c, off = divmod(r0, RC)
        if k == 0:
            y = jnp.dot(_unpacked(wt_s[WO_B]), ot_s[:, r0:r0 + n].astype(BF16), preferred_element_type=F32).T
        else:
            y = jnp.dot(ot_s[:, r0:r0 + n].T.astype(BF16), raw_s[WO_B], preferred_element_type=F32)
        xio_s[r0:r0 + n, :] = (x_s[c % 2][c // 2, off:off + n, :] + y).astype(BF16)
        out_copy(k).start()
    for k in range(len(pieces)):
        out_copy(k).wait()


@jax.jit
def pallas_interleave_layers__sliding_block__mha_block__prompt_kernel(A_x, A_wqkv, A_wo, B_x, B_wqkv, B_wo):
    del B_x
    out = pl.pallas_call(
        _kernel,
        out_shape=jax.ShapeDtypeStruct((S, D), BF16),
        in_specs=[pl.BlockSpec(memory_space=pl.ANY)] * 5,
        out_specs=pl.BlockSpec(memory_space=pl.ANY),
        scratch_shapes=[
            pltpu.VMEM((S, D), BF16),
            pltpu.VMEM((6, D, D), BF16),
            pltpu.VMEM((2, D, D), BF16),
            pltpu.VMEM((6, D // 2, D), U32),
            pltpu.VMEM((D // 2, D), U32),
            pltpu.VMEM((2, 8, D), F32),
            pltpu.VMEM((2, D, 128), F32),
            pltpu.VMEM((S, D), F32),
            pltpu.VMEM((H, S, 128), I8),
            pltpu.VMEM((H, 128, S), I8),
            pltpu.VMEM((H, 8, S), F32),
            pltpu.VMEM((D, S), F32),
            pltpu.VMEM((D, S), F32),
            pltpu.VMEM((8, 8, 128), F32),
            pltpu.VMEM((S, TQ), F32),
            pltpu.VMEM((KC, TQ), F32),
            pltpu.VMEM((DH, TQ), F32),
            pltpu.VMEM((8, TQ), F32),
            pltpu.SMEM((2,), F32),
            pltpu.SemaphoreType.DMA((8 + NRC,)),
            pltpu.VMEM((NX, RC, D), F32),
            pltpu.VMEM((NX, RC, D), F32),
            pltpu.VMEM((NX, RC // 2, D), U32),
            pltpu.VMEM((NX, RC // 2, D), U32),
        ],
        compiler_params=pltpu.CompilerParams(vmem_limit_bytes=110 * 1024 * 1024),
        name="fused4",
    )(A_x.reshape(S, D), A_wqkv, A_wo, B_wqkv, B_wo)
    return out.reshape(1, S, D)
```
